```python
import jax
import jax.numpy as jnp

def _softmax(x, axis=-1):
    return jax.nn.softmax(x, axis=axis)

def _gelu(x):
    return jax.nn.gelu(x, approximate=True)

def _silu(x):
    return jax.nn.silu(x)

def _sigmoid(x):
    return jax.nn.sigmoid(x)

def _layernorm(x, axis=-1, eps=1e-05):
    m = jnp.mean(x, axis=axis, keepdims=True)
    v = jnp.var(x, axis=axis, keepdims=True)
    return (x - m) / jnp.sqrt(v + eps)

def _scatter_add(tgt, idx, src, axis=0):
    return tgt.at[idx].add(src)

def _segment_sum(src, seg, n):
    return jax.ops.segment_sum(src, seg, n)

class _Rng:

    def __init__(self, key):
        self._k = key

    def _next(self):
        self._k, sub = jax.random.split(self._k)
        return sub

    def normal(self, shape):
        return jax.random.normal(self._next(), shape, dtype=jnp.bfloat16)

    def randint(self, lo, hi, shape):
        return jax.random.randint(self._next(), shape, lo, hi, dtype=jnp.int32)

    def uniform(self, shape, lo=0.0, hi=1.0):
        return jax.random.uniform(self._next(), shape, jnp.bfloat16, lo, hi)

    def permutation(self, n):
        return jax.random.permutation(self._next(), n)
kernel_name = 'adaLN_cond__memory_aug_recurrent_mem_tr__moe_arch_mod__prompt'

def setup_inputs():
    _rng = _Rng(jax.random.key(int.from_bytes(__import__("os").urandom(4), "little")))
    _w = lambda a: (lambda t: t.astype(jnp.bfloat16) if jnp.issubdtype(t.dtype, jnp.floating) else t)(jnp.asarray(a))

    def _A_setup():
        B, S, Dm = (1, 2048, 1024)
        H, Dh = (32, 128)
        M, seg = (8, 32)
        seg = min(seg, S)
        S = S // seg * seg
        return {'x': _w((lambda *s: _rng.normal(s) * 0.05)(B, S, Dm)), 'mem0': _w((lambda *s: _rng.normal(s) * 0.05)(B, M, Dm)), 'Wq': _w((lambda *s: _rng.normal(s) * 0.05)(Dm, H, Dh) * Dm ** (-0.5)), 'Wk': _w((lambda *s: _rng.normal(s) * 0.05)(Dm, H, Dh) * Dm ** (-0.5)), 'Wv': _w((lambda *s: _rng.normal(s) * 0.05)(Dm, H, Dh) * Dm ** (-0.5)), 'Wo': _w((lambda *s: _rng.normal(s) * 0.05)(H, Dh, Dm) * (H * Dh) ** (-0.5)), 'seg_len': seg}
    _A_in = _A_setup()

    def _B_setup():
        B, S, D, F, C = (1, 2048, 1024, 3584, 2)
        return {'x': _w((lambda *s: _rng.normal(s) * 0.05)(B, S, D)), 'w_r': _w((lambda *s: _rng.normal(s) * 0.05)(D)), 'w_gate': _w((lambda *s: _rng.normal(s) * 0.05)(D, F)), 'w_up': _w((lambda *s: _rng.normal(s) * 0.05)(D, F)), 'w_down': _w((lambda *s: _rng.normal(s) * 0.05)(F, D))}
    _B_in = _B_setup()
    return {'A_x': _A_in['x'], 'A_mem0': _A_in['mem0'], 'A_Wq': _A_in['Wq'], 'A_Wk': _A_in['Wk'], 'A_Wv': _A_in['Wv'], 'A_Wo': _A_in['Wo'], 'A_seg_len': _A_in['seg_len'], 'B_x': _B_in['x'], 'B_w_r': _B_in['w_r'], 'B_w_gate': _B_in['w_gate'], 'B_w_up': _B_in['w_up'], 'B_w_down': _B_in['w_down'], 'c': _w((lambda *s: _rng.normal(s) * 0.05)(1, 1024)), 'w_mod': _w((lambda *s: _rng.normal(s) * 0.05)(1024, 6 * 1024) * 1024 ** (-0.5))}

def reference(A_x, A_mem0, A_Wq, A_Wk, A_Wv, A_Wo, A_seg_len, B_x, B_w_r, B_w_gate, B_w_up, B_w_down, c, w_mod):

    def _A_ref(x, mem0, Wq, Wk, Wv, Wo, seg_len):
        B, S, Dm = x.shape
        H, Dh = (Wq.shape[1], Wq.shape[2])
        M = mem0.shape[1]
        scale = Dh ** (-0.5)
        n_seg = S // seg_len
        L = M + seg_len
        idx = jnp.arange(L)
        mask = (idx[:, None] < M) | (idx[:, None] >= idx[None, :])
        mem = mem0
        outs = []
        for s in range(n_seg):
            xs = x[:, s * seg_len:(s + 1) * seg_len, :].copy()
            h = jnp.concatenate([mem, xs], axis=1)
            q = jnp.einsum('btd,dhe->bhte', h, Wq)
            k = jnp.einsum('btd,dhe->bhte', h, Wk)
            v = jnp.einsum('btd,dhe->bhte', h, Wv)
            scores = jnp.einsum('bhqe,bhke->bhqk', q, k) * scale
            scores = jnp.where(mask[None, None], scores, -1000000000.0)
            p = _softmax(scores, axis=-1)
            o = jnp.einsum('bhqk,bhke->bhqe', p, v)
            o = jnp.einsum('bhte,hed->btd', o, Wo)
            mem = o[:, :M, :].copy()
            outs.append(o[:, M:, :])
        return jnp.concatenate(outs, axis=1)

    def _B_ref(x, w_r, w_gate, w_up, w_down):
        B, S, D = x.shape
        C = 2
        r = x @ w_r
        idx = jnp.argsort(-r, axis=-1)[:, :C]
        idx_e = jnp.repeat(idx.reshape(B, C, 1), D, axis=2)
        x_sel = jnp.take_along_axis(x, idx_e, axis=1)
        g = _silu(x_sel @ w_gate)
        u = x_sel @ w_up
        y = g * u @ w_down
        r_sel = _sigmoid(jnp.take_along_axis(r, idx, axis=1))
        y = y * r_sel.reshape(B, C, 1)
        b_off = (jnp.arange(B) * S).reshape(B, 1)
        flat_idx = (idx + b_off).reshape(B * C)
        zero = (x * 0.0).reshape(B * S, D)
        upd = _scatter_add(zero, flat_idx, y.reshape(B * C, D), axis=0)
        return x + upd.reshape(B, S, D)
    x = A_x
    mod = (_silu(c) @ w_mod).reshape(c.shape[0], 6, 1, -1)
    sa, ca, ga, sb, cb, gb = (mod[:, 0].copy(), mod[:, 1].copy(), mod[:, 2].copy(), mod[:, 3].copy(), mod[:, 4].copy(), mod[:, 5].copy())
    h = _layernorm(x, axis=-1) * (1 + ca) + sa
    x = x + ga * _A_ref(h, A_mem0, A_Wq, A_Wk, A_Wv, A_Wo, A_seg_len)
    h = _layernorm(x, axis=-1) * (1 + cb) + sb
    x = x + gb * _B_ref(h, B_w_r, B_w_gate, B_w_up, B_w_down)
    return x
```

```python
import jax
import jax.numpy as jnp
import jax.experimental.pallas as pl
import jax.experimental.pallas.tpu as pltpu

F32 = jnp.float32
BF16 = jnp.bfloat16
U32 = jnp.uint32

_NN = (((1,), (0,)), ((), ()))
_NT = (((1,), (1,)), ((), ()))


def _dot(a, b, dims=_NN):
    return jax.lax.dot_general(a, b, dims, preferred_element_type=F32)


def _w(v):
    return pltpu.bitcast(v, BF16)


def _rnd(v):
    return v.astype(BF16).astype(F32)


def _ln(v):
    m = jnp.mean(v, axis=-1, keepdims=True)
    d = v - m
    var = jnp.mean(d * d, axis=-1, keepdims=True)
    return d * jax.lax.rsqrt(var + 1e-05)


@jax.jit
def pallas_adaLN_cond__memory_aug_recurrent_mem_tr__moe_arch_mod__prompt_kernel(
    A_x: jax.Array,
    A_mem0: jax.Array,
    A_Wq: jax.Array,
    A_Wk: jax.Array,
    A_Wv: jax.Array,
    A_Wo: jax.Array,
    A_seg_len: jax.Array,
    B_x: jax.Array,
    B_w_r: jax.Array,
    B_w_gate: jax.Array,
    B_w_up: jax.Array,
    B_w_down: jax.Array,
    c: jax.Array,
    w_mod: jax.Array,
):
    B, S, D = A_x.shape
    _, H, E = A_Wq.shape
    M = A_mem0.shape[1]
    F = B_w_gate.shape[1]
    SEG = 32
    NSEG = S // SEG
    L = M + SEG
    HE = H * E
    scale = float(E) ** -0.5
    CH = 128
    NCH = D // CH
    NSLOT = 4
    RPD = H // 2

    def kernel(x_hbm, mem0_ref, wq_hbm, wk_hbm, wv_hbm, wo_hbm, wr_ref, c_ref, wmod_hbm,
               wg_hbm, wu_hbm, wd_hbm, out_hbm,
               x_v, wqkv, wo_v, wmod_v, wg_v, wu_v, wd_v, stage, x1_v, out_v, mem_v, mod_v, r_v,
               sems, ssem):
        cp_mod = pltpu.make_async_copy(wmod_hbm.bitcast(U32), wmod_v, sems.at[0])
        cp_x = pltpu.make_async_copy(x_hbm, x_v, sems.at[1])
        cp_wo = pltpu.make_async_copy(wo_hbm.bitcast(U32), wo_v, sems.at[2])
        cp_wg = pltpu.make_async_copy(wg_hbm.bitcast(U32), wg_v, sems.at[3])
        cp_wu = pltpu.make_async_copy(wu_hbm.bitcast(U32), wu_v, sems.at[4])
        cp_wd = pltpu.make_async_copy(wd_hbm.bitcast(U32), wd_v, sems.at[5])
        cp_out = pltpu.make_async_copy(out_v, out_hbm, sems.at[6])
        srcs = (wq_hbm, wk_hbm, wv_hbm)

        def stage_cp(j):
            wi, ci = divmod(j, NCH)
            src = srcs[wi].bitcast(U32).at[pl.ds(ci * CH * RPD, CH * RPD), :]
            return pltpu.make_async_copy(src, stage.at[j % NSLOT], ssem.at[j % NSLOT])

        cp_mod.start()
        cp_x.start()
        for j in range(NSLOT):
            stage_cp(j).start()
        for j in range(3 * NCH):
            wi, ci = divmod(j, NCH)
            slot = j % NSLOT
            stage_cp(j).wait()

            def cv(i, carry, slot=slot, wi=wi, ci=ci):
                base = pl.multiple_of(i * (16 * RPD), 16 * RPD)
                r2 = pl.multiple_of(ci * (CH // 2) + i * 8, 8)
                for hp in range(RPD):
                    a = stage[slot, pl.ds(base + hp, 8, stride=2 * RPD), :]
                    b = stage[slot, pl.ds(base + RPD + hp, 8, stride=2 * RPD), :]
                    lo = (a & jnp.uint32(0xFFFF)) | (b << 16)
                    hi = (a >> 16) | (b & jnp.uint32(0xFFFF0000))
                    wqkv[pl.ds(r2, 8), pl.ds(wi * HE + (2 * hp) * E, E)] = lo
                    wqkv[pl.ds(r2, 8), pl.ds(wi * HE + (2 * hp + 1) * E, E)] = hi
                return carry

            jax.lax.fori_loop(0, CH // 16, cv, 0)
            if j + NSLOT < 3 * NCH:
                stage_cp(j + NSLOT).start()
            if j == 3 * NCH - NSLOT:
                cp_wo.start()

        cp_mod.wait()
        cs = c_ref[...].astype(F32)
        cs = _rnd(cs * jax.nn.sigmoid(cs))
        mod_v[...] = _dot(jnp.broadcast_to(cs, (8, D)), _w(wmod_v[...]))
        mem_v[...] = mem0_ref[...].astype(F32)
        r_v[...] = jnp.zeros_like(r_v)
        cp_x.wait()
        cp_wo.wait()
        cp_wg.start()
        cp_wu.start()
        cp_wd.start()

        row = jax.lax.broadcasted_iota(jnp.int32, (L, L), 0)
        col = jax.lax.broadcasted_iota(jnp.int32, (L, L), 1)
        mask = (row < M) | (row >= col)
        lane = jax.lax.broadcasted_iota(jnp.int32, (SEG, 128), 1)

        def step(s, carry):
            r0 = pl.multiple_of(s * SEG, SEG)
            sa = mod_v[0:1, 0 * D:1 * D]
            ca = mod_v[0:1, 1 * D:2 * D]
            ga = mod_v[0:1, 2 * D:3 * D]
            sb = mod_v[0:1, 3 * D:4 * D]
            cb = mod_v[0:1, 4 * D:5 * D]
            gb = mod_v[0:1, 5 * D:6 * D]
            xs = x_v[pl.ds(r0, SEG), :].astype(F32)
            h = _ln(xs) * (1.0 + ca) + sa
            lhs = jnp.concatenate([mem_v[...], h], axis=0)
            qkv = _dot(lhs, _w(wqkv[...]))
            outs = []
            for hh in range(H):
                q = qkv[:, hh * E:(hh + 1) * E]
                k = qkv[:, HE + hh * E:HE + (hh + 1) * E]
                v = qkv[:, 2 * HE + hh * E:2 * HE + (hh + 1) * E]
                sc = _dot(q, k, _NT) * scale
                sc = jnp.where(mask, sc, -1000000000.0)
                e = jnp.exp(sc - jnp.max(sc, axis=-1, keepdims=True))
                p = e / jnp.sum(e, axis=-1, keepdims=True)
                outs.append(_dot(p, v))
            o = jnp.concatenate(outs, axis=1)
            y = _dot(o, _w(wo_v[...]))
            mem_v[...] = y[:M]
            x1 = _rnd(xs + _rnd(ga * y[M:]))
            h2 = _rnd(_ln(x1) * (1.0 + cb) + sb)
            wr = wr_ref[...].astype(F32).reshape(1, D)
            r = _rnd(jnp.sum(h2 * wr, axis=-1, keepdims=True))
            r_v[...] = jnp.where(lane == s, r, r_v[...])
            x1_v[pl.ds(r0, SEG), :] = x1
            out_v[pl.ds(r0, SEG), :] = (x1 + gb * h2).astype(BF16)
            return carry

        jax.lax.fori_loop(0, NSEG, step, 0)

        sb = mod_v[0:1, 3 * D:4 * D]
        cb = mod_v[0:1, 4 * D:5 * D]
        gb = mod_v[0:1, 5 * D:6 * D]
        tok = lane * SEG + jax.lax.broadcasted_iota(jnp.int32, (SEG, 128), 0)
        rv = jnp.where(lane < NSEG, r_v[...], -jnp.inf)
        m0 = jnp.max(rv)
        i0 = jnp.min(jnp.where(rv == m0, tok, S - 1))
        rv1 = jnp.where(tok == i0, -jnp.inf, rv)
        m1 = jnp.max(rv1)
        i1 = jnp.min(jnp.where(rv1 == m1, tok, S - 1))
        row8 = jax.lax.broadcasted_iota(jnp.int32, (8, D), 0)
        xa = x1_v[pl.ds(i0, 1), :]
        xb = x1_v[pl.ds(i1, 1), :]
        x1s = jnp.where(row8 == 0, xa, jnp.where(row8 == 1, xb, 0.0))
        h2s = _rnd(_ln(x1s) * (1.0 + cb) + sb)
        cp_wg.wait()
        cp_wu.wait()
        cp_wd.wait()
        g = _dot(h2s, _w(wg_v[...]))
        u = _dot(h2s, _w(wu_v[...]))
        y = _dot(g * jax.nn.sigmoid(g) * u, _w(wd_v[...]))
        rsel = jnp.where(row8 == 0, m0, m1)
        y = y * jax.nn.sigmoid(rsel)
        fix = x1s + gb * (h2s + y)
        row16 = jax.lax.broadcasted_iota(jnp.int32, (16, D), 0)
        for n, idx in enumerate((i0, i1)):
            g0 = pl.multiple_of((idx // 16) * 16, 16)
            blk = out_v[pl.ds(g0, 16), :].astype(F32)
            blk = jnp.where(row16 == idx - g0, fix[n:n + 1], blk)
            out_v[pl.ds(g0, 16), :] = blk.astype(BF16)
        cp_out.start()
        cp_out.wait()

    any_spec = pl.BlockSpec(memory_space=pl.ANY)
    vmem_spec = pl.BlockSpec(memory_space=pltpu.VMEM)
    out = pl.pallas_call(
        kernel,
        out_shape=jax.ShapeDtypeStruct((B * S, D), A_x.dtype),
        in_specs=[any_spec, vmem_spec, any_spec, any_spec, any_spec, any_spec, vmem_spec, vmem_spec,
                  any_spec, any_spec, any_spec, any_spec],
        out_specs=any_spec,
        scratch_shapes=[
            pltpu.VMEM((S, D), BF16),
            pltpu.VMEM((D // 2, 3 * HE), U32),
            pltpu.VMEM((HE // 2, D), U32),
            pltpu.VMEM((D // 2, 6 * D), U32),
            pltpu.VMEM((D // 2, F), U32),
            pltpu.VMEM((D // 2, F), U32),
            pltpu.VMEM((F // 2, D), U32),
            pltpu.VMEM((NSLOT, CH * RPD, E), U32),
            pltpu.VMEM((S, D), F32),
            pltpu.VMEM((S, D), BF16),
            pltpu.VMEM((M, D), F32),
            pltpu.VMEM((8, 6 * D), F32),
            pltpu.VMEM((SEG, 128), F32),
            pltpu.SemaphoreType.DMA((7,)),
            pltpu.SemaphoreType.DMA((NSLOT,)),
        ],
        compiler_params=pltpu.CompilerParams(vmem_limit_bytes=110 * 1024 * 1024),
    )(
        A_x.reshape(B * S, D), A_mem0.reshape(B * M, D),
        A_Wq.reshape(D * H, E), A_Wk.reshape(D * H, E), A_Wv.reshape(D * H, E),
        A_Wo.reshape(HE, D), B_w_r, c, w_mod, B_w_gate, B_w_up, B_w_down,
    )
    return out.reshape(B, S, D)
```

```python
import jax
import jax.numpy as jnp
import jax.experimental.pallas as pl
import jax.experimental.pallas.tpu as pltpu

F32 = jnp.float32
BF16 = jnp.bfloat16
U32 = jnp.uint32

_NN = (((1,), (0,)), ((), ()))
_NT = (((1,), (1,)), ((), ()))


def _dot(a, b, dims=_NN):
    return jax.lax.dot_general(a, b, dims, preferred_element_type=F32)


def _w(v):
    return pltpu.bitcast(v, BF16)


def _rnd(v):
    return v.astype(BF16).astype(F32)


def _ln(v):
    m = jnp.mean(v, axis=-1, keepdims=True)
    d = v - m
    var = jnp.mean(d * d, axis=-1, keepdims=True)
    return d * jax.lax.rsqrt(var + 1e-05)


@jax.jit
def pallas_adaLN_cond__memory_aug_recurrent_mem_tr__moe_arch_mod__prompt_kernel(
    A_x: jax.Array,
    A_mem0: jax.Array,
    A_Wq: jax.Array,
    A_Wk: jax.Array,
    A_Wv: jax.Array,
    A_Wo: jax.Array,
    A_seg_len: jax.Array,
    B_x: jax.Array,
    B_w_r: jax.Array,
    B_w_gate: jax.Array,
    B_w_up: jax.Array,
    B_w_down: jax.Array,
    c: jax.Array,
    w_mod: jax.Array,
):
    B, S, D = A_x.shape
    _, H, E = A_Wq.shape
    M = A_mem0.shape[1]
    F = B_w_gate.shape[1]
    SEG = 32
    NSEG = S // SEG
    L = M + SEG
    HE = H * E
    HP = H // 2
    scale = float(E) ** -0.5
    TPS = 24
    PRE = S - TPS * NSEG
    RING = 576
    SHIFT = RING - PRE
    LR = M + TPS
    XO = 2 * LR
    G = 8
    AHEAD = 3

    def kernel(x_hbm, mem0_ref, wq_hbm, wk_hbm, wv_hbm, wo_hbm, wr_ref, c_ref, wmod_hbm,
               wg_hbm, wu_hbm, wd_hbm, out_hbm,
               x_v, wqkv, wo_v, wmod_v, wg_v, wu_v, wd_v, ring, hpre, act_v, out_v, y_v, mod_v, r_v,
               sems, wsem):
        wmod32 = wmod_hbm.bitcast(U32)
        cp_mod1 = pltpu.make_async_copy(wmod32.at[:, pl.ds(0, 2 * D)], wmod_v.at[:, pl.ds(0, 2 * D)], sems.at[0])
        cp_mod2 = pltpu.make_async_copy(wmod32.at[:, pl.ds(2 * D, 4 * D)], wmod_v.at[:, pl.ds(2 * D, 4 * D)], sems.at[7])
        cp_x = pltpu.make_async_copy(x_hbm, x_v, sems.at[1])
        cp_wo = pltpu.make_async_copy(wo_hbm.bitcast(U32), wo_v, sems.at[2])
        cp_wg = pltpu.make_async_copy(wg_hbm.bitcast(U32), wg_v, sems.at[3])
        cp_wu = pltpu.make_async_copy(wu_hbm.bitcast(U32), wu_v, sems.at[4])
        cp_wd = pltpu.make_async_copy(wd_hbm.bitcast(U32), wd_v, sems.at[5])
        cp_out = pltpu.make_async_copy(out_v.at[pl.ds(SEG, S), :], out_hbm, sems.at[6])
        srcs = tuple(w.bitcast(U32) for w in (wq_hbm, wk_hbm, wv_hbm))

        def wcps(hp):
            return [pltpu.make_async_copy(srcs[wi].at[:, p, hp, :], wqkv.at[hp, wi, p], wsem.at[hp])
                    for wi in range(3) for p in range(2)]

        def repack(hp):
            for wi in range(3):
                a = wqkv[hp, wi, 0]
                b = wqkv[hp, wi, 1]
                wqkv[hp, wi, 0] = (a & jnp.uint32(0xFFFF)) | (b << 16)
                wqkv[hp, wi, 1] = (a >> 16) | (b & jnp.uint32(0xFFFF0000))

        def whead(hp, hb):
            return _w(jnp.concatenate([wqkv[hp, wi, hb] for wi in range(3)], axis=1))

        cp_mod1.start()
        cp_x.start()
        for hp in range(AHEAD):
            for cp in wcps(hp):
                cp.start()

        def mods(i):
            return mod_v[0:1, i * D:(i + 1) * D]

        cs = c_ref[...].astype(F32)
        cs = jnp.broadcast_to(_rnd(cs * jax.nn.sigmoid(cs)), (8, D))
        cp_mod1.wait()
        mod_v[:, :2 * D] = _dot(cs, _w(wmod_v[:, :2 * D]))
        cp_x.wait()

        def ada1(rows):
            return _ln(rows.astype(F32)) * (1.0 + mods(1)) + mods(0)

        def pre_ln(i, carry):
            r0 = pl.multiple_of(i * 64, 64)
            hpre[pl.ds(r0, 64), :] = ada1(x_v[pl.ds(r0, 64), :]).astype(BF16)
            return carry

        jax.lax.fori_loop(0, PRE // 64, pre_ln, 0)

        for cp in wcps(0):
            cp.wait()
        repack(0)

        def pre_proj(hp, carry):
            @pl.when(hp + AHEAD < HP)
            def _():
                for cp in wcps(hp + AHEAD):
                    cp.start()

            @pl.when(hp + AHEAD == HP)
            def _():
                cp_wo.start()
                cp_mod2.start()

            @pl.when(hp + 1 < HP)
            def _():
                for cp in wcps(hp + 1):
                    cp.wait()
                repack(hp + 1)

            for hb in range(2):
                col = pl.multiple_of((2 * hp + hb) * 3 * E, 3 * E)
                ring[pl.ds(SHIFT, PRE), pl.ds(col, 3 * E)] = _dot(hpre[...], whead(hp, hb))
            return carry

        jax.lax.fori_loop(0, HP, pre_proj, 0)

        cp_wg.start()
        cp_wu.start()
        cp_wd.start()
        cp_mod2.wait()
        mod_v[:, 2 * D:] = _dot(cs, _w(wmod_v[:, 2 * D:]))
        cp_wo.wait()

        row = jax.lax.broadcasted_iota(jnp.int32, (L, L), 0)
        col = jax.lax.broadcasted_iota(jnp.int32, (L, L), 1)
        mask = (row < M) | (row >= col)
        lane = jax.lax.broadcasted_iota(jnp.int32, (SEG, 128), 1)

        def pre(s, slot):
            r0 = pl.multiple_of(PRE + s * TPS, 8)
            act_v[pl.ds(pl.multiple_of(slot * LR + M, 8), TPS), :] = ada1(x_v[pl.ds(r0, TPS), :])

        def post(s):
            rx = pl.multiple_of(jnp.maximum(s, 0) * SEG, SEG)
            r0 = pl.multiple_of((s + 1) * SEG, SEG)
            xs = x_v[pl.ds(rx, SEG), :].astype(F32)
            x1 = _rnd(xs + _rnd(mods(2) * y_v[...]))
            h2 = _rnd(_ln(x1) * (1.0 + mods(4)) + mods(3))
            wr = wr_ref[...].astype(F32).reshape(1, D)
            r = _rnd(jnp.sum(h2 * wr, axis=-1, keepdims=True))
            r_v[...] = jnp.where(lane == s, r, r_v[...])
            act_v[pl.ds(XO + r0, SEG), :] = x1
            out_v[pl.ds(r0, SEG), :] = (x1 + mods(5) * h2).astype(BF16)

        def step(s, carry):
            cur = pl.multiple_of((s % 2) * LR, 8)
            nxt = 1 - s % 2
            wrow = pl.multiple_of((s * TPS) % RING, 8)
            rrow = pl.multiple_of((s * SEG + SHIFT) % RING, 8)
            qkv, p, o = {}, {}, {}
            y = None
            for t in range(H + 3):
                if t < H:
                    cols = pl.ds(t * 3 * E, 3 * E)
                    res = _dot(act_v[pl.ds(cur, LR), :], whead(t // 2, t % 2))
                    ring[pl.ds(wrow, TPS), cols] = res[M:]
                    qkv[t] = jnp.concatenate([res[:M], ring[pl.ds(rrow, SEG), cols]], axis=0)
                if t == 1:
                    post(s - 1)
                if t == 3:
                    pre(jnp.minimum(s + 1, NSEG - 1), nxt)
                hh = t - 1
                if 0 <= hh < H:
                    sc = _dot(qkv[hh][:, :E], qkv[hh][:, E:2 * E], _NT) * scale
                    sc = jnp.where(mask, sc, -1000000000.0)
                    e = jnp.exp(sc - jnp.max(sc, axis=-1, keepdims=True))
                    p[hh] = e / jnp.sum(e, axis=-1, keepdims=True)
                hh = t - 3
                if 0 <= hh < H:
                    o[hh] = _dot(p[hh], qkv[hh][:, 2 * E:])
                for g in {H - 1: [0], H: [1], H + 3 - 1: [2, 3]}.get(t, []):
                    og = jnp.concatenate([o[i] for i in range(g * G, (g + 1) * G)], axis=1)
                    yg = _dot(og, _w(wo_v[g * G * E // 2:(g + 1) * G * E // 2, :]))
                    y = yg if y is None else y + yg
            act_v[pl.ds(pl.multiple_of(nxt * LR, 8), M), :] = y[:M]
            y_v[...] = y[M:]
            return carry

        r_v[...] = jnp.zeros_like(r_v)
        y_v[...] = jnp.zeros_like(y_v)
        act_v[:M, :] = mem0_ref[...].astype(F32)
        pre(0, 0)
        jax.lax.fori_loop(0, NSEG, step, 0)
        post(NSEG - 1)

        sb, cb, gb = mods(3), mods(4), mods(5)
        tok = lane * SEG + jax.lax.broadcasted_iota(jnp.int32, (SEG, 128), 0)
        rv = jnp.where(lane < NSEG, r_v[...], -jnp.inf)
        m0 = jnp.max(rv)
        i0 = jnp.min(jnp.where(rv == m0, tok, S - 1))
        rv1 = jnp.where(tok == i0, -jnp.inf, rv)
        m1 = jnp.max(rv1)
        i1 = jnp.min(jnp.where(rv1 == m1, tok, S - 1))
        row8 = jax.lax.broadcasted_iota(jnp.int32, (8, D), 0)
        xa = act_v[pl.ds(XO + SEG + i0, 1), :]
        xb = act_v[pl.ds(XO + SEG + i1, 1), :]
        x1s = jnp.where(row8 == 0, xa, jnp.where(row8 == 1, xb, 0.0))
        h2s = _rnd(_ln(x1s) * (1.0 + cb) + sb)
        cp_wg.wait()
        cp_wu.wait()
        cp_wd.wait()
        g = _dot(h2s, _w(wg_v[...]))
        u = _dot(h2s, _w(wu_v[...]))
        y = _dot(g * jax.nn.sigmoid(g) * u, _w(wd_v[...]))
        rsel = jnp.where(row8 == 0, m0, m1)
        y = y * jax.nn.sigmoid(rsel)
        fix = x1s + gb * (h2s + y)
        row16 = jax.lax.broadcasted_iota(jnp.int32, (16, D), 0)
        for n, idx in enumerate((i0, i1)):
            g0 = pl.multiple_of((idx // 16) * 16, 16)
            blk = out_v[pl.ds(g0 + SEG, 16), :].astype(F32)
            blk = jnp.where(row16 == idx - g0, fix[n:n + 1], blk)
            out_v[pl.ds(g0 + SEG, 16), :] = blk.astype(BF16)
        cp_out.start()
        cp_out.wait()

    any_spec = pl.BlockSpec(memory_space=pl.ANY)
    vmem_spec = pl.BlockSpec(memory_space=pltpu.VMEM)
    out = pl.pallas_call(
        kernel,
        out_shape=jax.ShapeDtypeStruct((B * S, D), A_x.dtype),
        in_specs=[any_spec, vmem_spec, any_spec, any_spec, any_spec, any_spec, vmem_spec, vmem_spec,
                  any_spec, any_spec, any_spec, any_spec],
        out_specs=any_spec,
        scratch_shapes=[
            pltpu.VMEM((S, D), BF16),
            pltpu.VMEM((HP, 3, 2, D // 2, E), U32),
            pltpu.VMEM((HE // 2, D), U32),
            pltpu.VMEM((D // 2, 6 * D), U32),
            pltpu.VMEM((D // 2, F), U32),
            pltpu.VMEM((D // 2, F), U32),
            pltpu.VMEM((F // 2, D), U32),
            pltpu.VMEM((RING, 3 * HE), F32),
            pltpu.VMEM((PRE, D), BF16),
            pltpu.VMEM((XO + S + SEG, D), F32),
            pltpu.VMEM((S + SEG, D), BF16),
            pltpu.VMEM((SEG, D), F32),
            pltpu.VMEM((8, 6 * D), F32),
            pltpu.VMEM((SEG, 128), F32),
            pltpu.SemaphoreType.DMA((8,)),
            pltpu.SemaphoreType.DMA((HP,)),
        ],
        compiler_params=pltpu.CompilerParams(vmem_limit_bytes=120 * 1024 * 1024),
    )(
        A_x.reshape(B * S, D), A_mem0.reshape(B * M, D),
        A_Wq.reshape(D // 2, 2, H, E), A_Wk.reshape(D // 2, 2, H, E), A_Wv.reshape(D // 2, 2, H, E),
        A_Wo.reshape(HE, D), B_w_r, c, w_mod, B_w_gate, B_w_up, B_w_down,
    )
    return out.reshape(B, S, D)
```

```python
import jax
import jax.numpy as jnp
import jax.experimental.pallas as pl
import jax.experimental.pallas.tpu as pltpu

F32 = jnp.float32
BF16 = jnp.bfloat16
U32 = jnp.uint32

_NN = (((1,), (0,)), ((), ()))
_NT = (((1,), (1,)), ((), ()))


def _dot(a, b, dims=_NN):
    return jax.lax.dot_general(a, b, dims, preferred_element_type=F32)


def _w(v):
    return pltpu.bitcast(v, BF16)


def _rnd(v):
    return v.astype(BF16).astype(F32)


def _ln(v):
    m = jnp.mean(v, axis=-1, keepdims=True)
    d = v - m
    var = jnp.mean(d * d, axis=-1, keepdims=True)
    return d * jax.lax.rsqrt(var + 1e-05)


@jax.jit
def pallas_adaLN_cond__memory_aug_recurrent_mem_tr__moe_arch_mod__prompt_kernel(
    A_x: jax.Array,
    A_mem0: jax.Array,
    A_Wq: jax.Array,
    A_Wk: jax.Array,
    A_Wv: jax.Array,
    A_Wo: jax.Array,
    A_seg_len: jax.Array,
    B_x: jax.Array,
    B_w_r: jax.Array,
    B_w_gate: jax.Array,
    B_w_up: jax.Array,
    B_w_down: jax.Array,
    c: jax.Array,
    w_mod: jax.Array,
):
    B, S, D = A_x.shape
    _, H, E = A_Wq.shape
    M = A_mem0.shape[1]
    F = B_w_gate.shape[1]
    SEG = 32
    NSEG = S // SEG
    L = M + SEG
    HE = H * E
    HP = H // 2
    scale = float(E) ** -0.5
    TPS = 24
    PRE = S - TPS * NSEG
    RING = 576
    SHIFT = RING - PRE
    LR = M + TPS
    XO = 2 * LR
    G = 8
    OB = 8

    def kernel(x_hbm, mem0_ref, wq_hbm, wk_hbm, wv_hbm, wo_hbm, wr_ref, c_ref, wmod_hbm,
               wg_hbm, wu_hbm, wd_hbm, out_hbm,
               x_v, wqkv, wo_v, wmod_v, wg_v, wu_v, wd_v, ring, hpre, act_v, out_v, y_v, mod_v, r_v,
               sems, wsem):
        wmod32 = wmod_hbm.bitcast(U32)
        cp_mod1 = pltpu.make_async_copy(wmod32.at[:, pl.ds(0, 2 * D)], wmod_v.at[:, pl.ds(0, 2 * D)], sems.at[0])
        cp_mod2 = pltpu.make_async_copy(wmod32.at[:, pl.ds(2 * D, 4 * D)], wmod_v.at[:, pl.ds(2 * D, 4 * D)], sems.at[7])
        cp_x1 = pltpu.make_async_copy(x_hbm.at[pl.ds(0, PRE), :], x_v.at[pl.ds(0, PRE), :], sems.at[1])
        cp_x2 = pltpu.make_async_copy(x_hbm.at[pl.ds(PRE, S - PRE), :], x_v.at[pl.ds(PRE, S - PRE), :], sems.at[8])
        cp_wo = pltpu.make_async_copy(wo_hbm.bitcast(U32), wo_v, sems.at[2])
        cp_wg = pltpu.make_async_copy(wg_hbm.bitcast(U32), wg_v, sems.at[3])
        cp_wu = pltpu.make_async_copy(wu_hbm.bitcast(U32), wu_v, sems.at[4])
        cp_wd = pltpu.make_async_copy(wd_hbm.bitcast(U32), wd_v, sems.at[5])

        def cp_out(r0, n):
            return pltpu.make_async_copy(out_v.at[pl.ds(SEG + r0, n), :], out_hbm.at[pl.ds(r0, n), :], sems.at[6])

        srcs = tuple(w.bitcast(U32) for w in (wq_hbm, wk_hbm, wv_hbm))

        def wcps(hp):
            return [pltpu.make_async_copy(srcs[wi].at[:, p, hp, :], wqkv.at[hp, wi, p], wsem.at[hp])
                    for wi in range(3) for p in range(2)]

        def repack(hp):
            for wi in range(3):
                a = wqkv[hp, wi, 0]
                b = wqkv[hp, wi, 1]
                wqkv[hp, wi, 0] = (a & jnp.uint32(0xFFFF)) | (b << 16)
                wqkv[hp, wi, 1] = (a >> 16) | (b & jnp.uint32(0xFFFF0000))

        def whead(hp, hb):
            return _w(jnp.concatenate([wqkv[hp, wi, hb] for wi in range(3)], axis=1))

        cp_mod1.start()
        cp_x1.start()
        wqkv[HP] = jnp.zeros(wqkv.shape[1:], U32)

        def mods(i):
            return mod_v[0:1, i * D:(i + 1) * D]

        cs = c_ref[...].astype(F32)
        cs = jnp.broadcast_to(_rnd(cs * jax.nn.sigmoid(cs)), (8, D))
        cp_mod1.wait()
        for cp in wcps(0):
            cp.start()
        cp_x1.wait()
        mod_v[:, :2 * D] = _dot(cs, _w(wmod_v[:, :2 * D]))
        for cp in wcps(1):
            cp.start()

        def ada1(rows):
            return _ln(rows.astype(F32)) * (1.0 + mods(1)) + mods(0)

        def pre_ln(i, carry):
            r0 = pl.multiple_of(i * 64, 64)
            hpre[pl.ds(r0, 64), :] = ada1(x_v[pl.ds(r0, 64), :]).astype(BF16)
            return carry

        jax.lax.fori_loop(0, PRE // 64, pre_ln, 0)

        for cp in wcps(0):
            cp.wait()
        repack(0)

        def pre_proj(hp, carry):
            @pl.when(2 * hp + 2 < HP)
            def _():
                for cp in wcps(2 * hp + 2) + wcps(2 * hp + 3):
                    cp.start()

            for at, cps in ((HP // 2 - 1, (cp_wo, cp_x2)), (HP // 2 + 2, (cp_mod2,))):
                @pl.when(hp == at)
                def _():
                    for cp in cps:
                        cp.start()

            @pl.when(hp + 1 < HP)
            def _():
                for cp in wcps(hp + 1):
                    cp.wait()

            repack(hp + 1)
            for hb in range(2):
                col = pl.multiple_of((2 * hp + hb) * 3 * E, 3 * E)
                ring[pl.ds(SHIFT, PRE), pl.ds(col, 3 * E)] = _dot(hpre[...], whead(hp, hb))
            return carry

        jax.lax.fori_loop(0, HP, pre_proj, 0)

        cp_wg.start()
        cp_wu.start()
        cp_wd.start()
        cp_mod2.wait()
        mod_v[:, 2 * D:] = _dot(cs, _w(wmod_v[:, 2 * D:]))
        cp_wo.wait()
        cp_x2.wait()

        row = jax.lax.broadcasted_iota(jnp.int32, (L, L), 0)
        col = jax.lax.broadcasted_iota(jnp.int32, (L, L), 1)
        mask = (row < M) | (row >= col)
        lane = jax.lax.broadcasted_iota(jnp.int32, (SEG, 128), 1)

        def pre(s, slot):
            r0 = pl.multiple_of(PRE + s * TPS, 8)
            act_v[pl.ds(pl.multiple_of(slot * LR + M, 8), TPS), :] = ada1(x_v[pl.ds(r0, TPS), :])

        def post(s):
            rx = pl.multiple_of(jnp.maximum(s, 0) * SEG, SEG)
            r0 = pl.multiple_of((s + 1) * SEG, SEG)
            xs = x_v[pl.ds(rx, SEG), :].astype(F32)
            x1 = _rnd(xs + _rnd(mods(2) * y_v[...]))
            h2 = _rnd(_ln(x1) * (1.0 + mods(4)) + mods(3))
            wr = wr_ref[...].astype(F32).reshape(1, D)
            r = _rnd(jnp.sum(h2 * wr, axis=-1, keepdims=True))
            r_v[...] = jnp.where(lane == s, r, r_v[...])
            act_v[pl.ds(XO + r0, SEG), :] = x1
            out_v[pl.ds(r0, SEG), :] = (x1 + mods(5) * h2).astype(BF16)

        def step(s, carry):
            cur = pl.multiple_of((s % 2) * LR, 8)
            nxt = 1 - s % 2
            wrow = pl.multiple_of((s * TPS) % RING, 8)
            rrow = pl.multiple_of((s * SEG + SHIFT) % RING, 8)
            qkv, p, o = {}, {}, {}
            y = None
            for t in range(H + 3):
                if t < H:
                    cols = pl.ds(t * 3 * E, 3 * E)
                    res = _dot(act_v[pl.ds(cur, LR), :], whead(t // 2, t % 2))
                    ring[pl.ds(wrow, TPS), cols] = res[M:]
                    qkv[t] = jnp.concatenate([res[:M], ring[pl.ds(rrow, SEG), cols]], axis=0)
                if t == 1:
                    post(s - 1)
                if t == 3:
                    pre(jnp.minimum(s + 1, NSEG - 1), nxt)
                hh = t - 1
                if 0 <= hh < H:
                    sc = _dot(qkv[hh][:, :E], qkv[hh][:, E:2 * E], _NT) * scale
                    sc = jnp.where(mask, sc, -1000000000.0)
                    e = jnp.exp(sc - jnp.max(sc, axis=-1, keepdims=True))
                    p[hh] = e / jnp.sum(e, axis=-1, keepdims=True)
                hh = t - 3
                if 0 <= hh < H:
                    o[hh] = _dot(p[hh], qkv[hh][:, 2 * E:])
                for g in {H - 1: [0], H: [1], H + 3 - 1: [2, 3]}.get(t, []):
                    og = jnp.concatenate([o[i] for i in range(g * G, (g + 1) * G)], axis=1)
                    yg = _dot(og, _w(wo_v[g * G * E // 2:(g + 1) * G * E // 2, :]))
                    y = yg if y is None else y + yg
            act_v[pl.ds(pl.multiple_of(nxt * LR, 8), M), :] = y[:M]
            y_v[...] = y[M:]

            @pl.when((s % OB == 0) & (s > 0))
            def _():
                cp_out(pl.multiple_of((s - OB) * SEG, OB * SEG), OB * SEG).start()

            return carry

        r_v[...] = jnp.zeros_like(r_v)
        y_v[...] = jnp.zeros_like(y_v)
        act_v[:M, :] = mem0_ref[...].astype(F32)
        pre(0, 0)
        jax.lax.fori_loop(0, NSEG, step, 0)
        post(NSEG - 1)
        cp_out((NSEG - OB) * SEG, OB * SEG).start()

        sb, cb, gb = mods(3), mods(4), mods(5)
        tok = lane * SEG + jax.lax.broadcasted_iota(jnp.int32, (SEG, 128), 0)
        rv = jnp.where(lane < NSEG, r_v[...], -jnp.inf)
        m0 = jnp.max(rv)
        i0 = jnp.min(jnp.where(rv == m0, tok, S - 1))
        rv1 = jnp.where(tok == i0, -jnp.inf, rv)
        m1 = jnp.max(rv1)
        i1 = jnp.min(jnp.where(rv1 == m1, tok, S - 1))
        row8 = jax.lax.broadcasted_iota(jnp.int32, (8, D), 0)
        xa = act_v[pl.ds(XO + SEG + i0, 1), :]
        xb = act_v[pl.ds(XO + SEG + i1, 1), :]
        x1s = jnp.where(row8 == 0, xa, jnp.where(row8 == 1, xb, 0.0))
        h2s = _rnd(_ln(x1s) * (1.0 + cb) + sb)
        cp_wg.wait()
        cp_wu.wait()
        cp_wd.wait()
        g = _dot(h2s, _w(wg_v[...]))
        u = _dot(h2s, _w(wu_v[...]))
        y = _dot(g * jax.nn.sigmoid(g) * u, _w(wd_v[...]))
        rsel = jnp.where(row8 == 0, m0, m1)
        y = y * jax.nn.sigmoid(rsel)
        fix = x1s + gb * (h2s + y)
        row16 = jax.lax.broadcasted_iota(jnp.int32, (16, D), 0)
        for n, idx in enumerate((i0, i1)):
            g0 = pl.multiple_of((idx // 16) * 16, 16)
            blk = out_v[pl.ds(g0 + SEG, 16), :].astype(F32)
            blk = jnp.where(row16 == idx - g0, fix[n:n + 1], blk)
            out_v[pl.ds(g0 + SEG, 16), :] = blk.astype(BF16)
        cp_out(0, S).wait()
        g0 = pl.multiple_of((i0 // 16) * 16, 16)
        g1 = pl.multiple_of((i1 // 16) * 16, 16)
        cp_out(g0, 16).start()

        @pl.when(g0 != g1)
        def _():
            cp_out(g1, 16).start()

        cp_out(g0, 16).wait()

        @pl.when(g0 != g1)
        def _():
            cp_out(g1, 16).wait()

    any_spec = pl.BlockSpec(memory_space=pl.ANY)
    vmem_spec = pl.BlockSpec(memory_space=pltpu.VMEM)
    out = pl.pallas_call(
        kernel,
        out_shape=jax.ShapeDtypeStruct((B * S, D), A_x.dtype),
        in_specs=[any_spec, vmem_spec, any_spec, any_spec, any_spec, any_spec, vmem_spec, vmem_spec,
                  any_spec, any_spec, any_spec, any_spec],
        out_specs=any_spec,
        scratch_shapes=[
            pltpu.VMEM((S, D), BF16),
            pltpu.VMEM((HP + 1, 3, 2, D // 2, E), U32),
            pltpu.VMEM((HE // 2, D), U32),
            pltpu.VMEM((D // 2, 6 * D), U32),
            pltpu.VMEM((D // 2, F), U32),
            pltpu.VMEM((D // 2, F), U32),
            pltpu.VMEM((F // 2, D), U32),
            pltpu.VMEM((RING, 3 * HE), F32),
            pltpu.VMEM((PRE, D), BF16),
            pltpu.VMEM((XO + S + SEG, D), F32),
            pltpu.VMEM((S + SEG, D), BF16),
            pltpu.VMEM((SEG, D), F32),
            pltpu.VMEM((8, 6 * D), F32),
            pltpu.VMEM((SEG, 128), F32),
            pltpu.SemaphoreType.DMA((9,)),
            pltpu.SemaphoreType.DMA((HP,)),
        ],
        compiler_params=pltpu.CompilerParams(vmem_limit_bytes=120 * 1024 * 1024),
    )(
        A_x.reshape(B * S, D), A_mem0.reshape(B * M, D),
        A_Wq.reshape(D // 2, 2, H, E), A_Wk.reshape(D // 2, 2, H, E), A_Wv.reshape(D // 2, 2, H, E),
        A_Wo.reshape(HE, D), B_w_r, c, w_mod, B_w_gate, B_w_up, B_w_down,
    )
    return out.reshape(B, S, D)
```

```python
import jax
import jax.numpy as jnp
import jax.experimental.pallas as pl
import jax.experimental.pallas.tpu as pltpu

F32 = jnp.float32
BF16 = jnp.bfloat16
U32 = jnp.uint32

_NN = (((1,), (0,)), ((), ()))
_NT = (((1,), (1,)), ((), ()))


def _dot(a, b, dims=_NN):
    return jax.lax.dot_general(a, b, dims, preferred_element_type=F32)


def _w(v):
    return pltpu.bitcast(v, BF16)


def _rnd(v):
    return v.astype(BF16).astype(F32)


def _ln(v):
    m = jnp.mean(v, axis=-1, keepdims=True)
    d = v - m
    var = jnp.mean(d * d, axis=-1, keepdims=True)
    return d * jax.lax.rsqrt(var + 1e-05)


@jax.jit
def pallas_adaLN_cond__memory_aug_recurrent_mem_tr__moe_arch_mod__prompt_kernel(
    A_x: jax.Array,
    A_mem0: jax.Array,
    A_Wq: jax.Array,
    A_Wk: jax.Array,
    A_Wv: jax.Array,
    A_Wo: jax.Array,
    A_seg_len: jax.Array,
    B_x: jax.Array,
    B_w_r: jax.Array,
    B_w_gate: jax.Array,
    B_w_up: jax.Array,
    B_w_down: jax.Array,
    c: jax.Array,
    w_mod: jax.Array,
):
    B, S, D = A_x.shape
    _, H, E = A_Wq.shape
    M = A_mem0.shape[1]
    F = B_w_gate.shape[1]
    SEG = 32
    NSEG = S // SEG
    L = M + SEG
    HE = H * E
    HP = H // 2
    scale = float(E) ** -0.5
    TPS = 24
    PRE = S - TPS * NSEG
    RING = 576
    SHIFT = RING - PRE
    LR = M + TPS
    XO = 2 * LR
    LAGS = (1, 2, 4)
    ORDER = ('qkv', 'misc', 'qk', 'sm', 'pv', 'wo')
    POST_AT = 1
    PRE_AT = 3
    WO_AT = {31: [(0, 8)], 32: [(8, 16)], 35: [(16, 24), (24, 32)]}
    FLAGS = {'XLA_TPU_EVENLY_DISTRIBUTE_CRITICAL_NODES': True}
    LB = 2
    KB = 0
    OB = 8

    def kernel(x_hbm, mem0_ref, wq_hbm, wk_hbm, wv_hbm, wo_hbm, wr_ref, c_ref, wmod_hbm,
               wg_hbm, wu_hbm, wd_hbm, out_hbm,
               x_v, wqkv, wo_v, wmod_v, wg_v, wu_v, wd_v, ring, hpre, act_v, out_v, y_v, mod_v, r_v,
               sems, wsem):
        wmod32 = wmod_hbm.bitcast(U32)
        cp_mod1 = pltpu.make_async_copy(wmod32.at[:, pl.ds(0, 2 * D)], wmod_v.at[:, pl.ds(0, 2 * D)], sems.at[0])
        cp_mod2 = pltpu.make_async_copy(wmod32.at[:, pl.ds(2 * D, 4 * D)], wmod_v.at[:, pl.ds(2 * D, 4 * D)], sems.at[7])
        cp_x1 = pltpu.make_async_copy(x_hbm.at[pl.ds(0, PRE), :], x_v.at[pl.ds(0, PRE), :], sems.at[1])
        cp_x2 = pltpu.make_async_copy(x_hbm.at[pl.ds(PRE, S - PRE), :], x_v.at[pl.ds(PRE, S - PRE), :], sems.at[8])
        cp_wo = pltpu.make_async_copy(wo_hbm.bitcast(U32), wo_v, sems.at[2])
        cp_wg = pltpu.make_async_copy(wg_hbm.bitcast(U32), wg_v, sems.at[3])
        cp_wu = pltpu.make_async_copy(wu_hbm.bitcast(U32), wu_v, sems.at[4])
        cp_wd = pltpu.make_async_copy(wd_hbm.bitcast(U32), wd_v, sems.at[5])

        def cp_out(r0, n):
            return pltpu.make_async_copy(out_v.at[pl.ds(SEG + r0, n), :], out_hbm.at[pl.ds(r0, n), :], sems.at[6])

        srcs = tuple(w.bitcast(U32) for w in (wq_hbm, wk_hbm, wv_hbm))

        def wcps(hp):
            return [pltpu.make_async_copy(srcs[wi].at[:, p, hp, :], wqkv.at[hp, wi, p], wsem.at[hp])
                    for wi in range(3) for p in range(2)]

        def repack(hp):
            for wi in range(3):
                a = wqkv[hp, wi, 0]
                b = wqkv[hp, wi, 1]
                wqkv[hp, wi, 0] = (a & jnp.uint32(0xFFFF)) | (b << 16)
                wqkv[hp, wi, 1] = (a >> 16) | (b & jnp.uint32(0xFFFF0000))

        def whead(hp, hb):
            return _w(jnp.concatenate([wqkv[hp, wi, hb] for wi in range(3)], axis=1))

        cp_mod1.start()
        cp_x1.start()
        wqkv[HP] = jnp.zeros(wqkv.shape[1:], U32)

        def mods(i):
            return mod_v[0:1, i * D:(i + 1) * D]

        cs = c_ref[...].astype(F32)
        cs = jnp.broadcast_to(_rnd(cs * jax.nn.sigmoid(cs)), (8, D))
        cp_mod1.wait()
        for cp in wcps(0):
            cp.start()
        cp_x1.wait()
        mod_v[:, :2 * D] = _dot(cs, _w(wmod_v[:, :2 * D]))
        for cp in wcps(1):
            cp.start()

        def ada1(rows):
            return _ln(rows.astype(F32)) * (1.0 + mods(1)) + mods(0)

        def pre_ln(i, carry):
            r0 = pl.multiple_of(i * 64, 64)
            hpre[pl.ds(r0, 64), :] = ada1(x_v[pl.ds(r0, 64), :]).astype(BF16)
            return carry

        jax.lax.fori_loop(0, PRE // 64, pre_ln, 0)

        for cp in wcps(0):
            cp.wait()
        repack(0)

        def pre_proj(hp, carry):
            @pl.when(2 * hp + 2 < HP)
            def _():
                for cp in wcps(2 * hp + 2) + wcps(2 * hp + 3):
                    cp.start()

            for at, cps in ((HP // 2 - 1, (cp_wo, cp_x2)), (HP // 2 + 2, (cp_mod2,))):
                @pl.when(hp == at)
                def _():
                    for cp in cps:
                        cp.start()

            @pl.when(hp + 1 < HP)
            def _():
                for cp in wcps(hp + 1):
                    cp.wait()

            repack(hp + 1)
            for hb in range(2):
                col = pl.multiple_of((2 * hp + hb) * 3 * E, 3 * E)
                ring[pl.ds(SHIFT, PRE), pl.ds(col, 3 * E)] = _dot(hpre[...], whead(hp, hb))
            return carry

        jax.lax.fori_loop(0, HP, pre_proj, 0)

        cp_wg.start()
        cp_wu.start()
        cp_wd.start()
        cp_mod2.wait()
        mod_v[:, 2 * D:] = _dot(cs, _w(wmod_v[:, 2 * D:]))
        cp_wo.wait()
        cp_x2.wait()

        row = jax.lax.broadcasted_iota(jnp.int32, (L, L), 0)
        col = jax.lax.broadcasted_iota(jnp.int32, (L, L), 1)
        mask = (row < M) | (row >= col)
        lane = jax.lax.broadcasted_iota(jnp.int32, (SEG, 128), 1)

        def pre(s, slot):
            r0 = pl.multiple_of(PRE + s * TPS, 8)
            act_v[pl.ds(pl.multiple_of(slot * LR + M, 8), TPS), :] = ada1(x_v[pl.ds(r0, TPS), :])

        def post(s):
            rx = pl.multiple_of(jnp.maximum(s, 0) * SEG, SEG)
            r0 = pl.multiple_of((s + 1) * SEG, SEG)
            xs = x_v[pl.ds(rx, SEG), :].astype(F32)
            x1 = _rnd(xs + _rnd(mods(2) * y_v[...]))
            h2 = _rnd(_ln(x1) * (1.0 + mods(4)) + mods(3))
            wr = wr_ref[...].astype(F32).reshape(1, D)
            r = _rnd(jnp.sum(h2 * wr, axis=-1, keepdims=True))
            r_v[...] = jnp.where(lane == s, r, r_v[...])
            act_v[pl.ds(XO + r0, SEG), :] = x1
            out_v[pl.ds(r0, SEG), :] = (x1 + mods(5) * h2).astype(BF16)

        def step(s, carry):
            cur = pl.multiple_of((s % 2) * LR, 8)
            nxt = 1 - s % 2
            wrow = pl.multiple_of((s * TPS) % RING, 8)
            rrow = pl.multiple_of((s * SEG + SHIFT) % RING, 8)
            qkv, sc, p, o = {}, {}, {}, {}
            lhs = act_v[pl.ds(cur, LR), :].astype(BF16) if LB == 2 else None
            ys = [None]

            def st_qkv(t):
                cols = pl.ds(t * 3 * E, 3 * E)
                res = _dot(lhs if LB == 2 else act_v[pl.ds(cur, LR), :].astype(BF16 if LB else F32), whead(t // 2, t % 2))
                ring[pl.ds(wrow, TPS), cols] = res[M:]
                qkv[t] = jnp.concatenate([res[:M], ring[pl.ds(rrow, SEG), cols]], axis=0)

            def st_qk(hh):
                sc[hh] = _dot(qkv[hh][:, :E], qkv[hh][:, E:2 * E].astype(BF16 if KB & 1 else F32), _NT)

            def st_sm(hh):
                z = jnp.where(mask, sc[hh] * scale, -1000000000.0)
                e = jnp.exp(z - jnp.max(z, axis=-1, keepdims=True))
                p[hh] = e / jnp.sum(e, axis=-1, keepdims=True)

            def st_pv(hh):
                o[hh] = _dot(p[hh], qkv[hh][:, 2 * E:].astype(BF16 if KB & 2 else F32))

            def st_wo(g):
                og = jnp.concatenate([o[i] for i in range(g[0], g[1])], axis=1)
                yg = _dot(og, _w(wo_v[g[0] * E // 2:g[1] * E // 2, :]))
                ys[0] = yg if ys[0] is None else ys[0] + yg

            for t in range(H + LAGS[2] + 1):
                for name in ORDER:
                    if name == "qkv" and t < H:
                        st_qkv(t)
                    if name == "misc":
                        if t == POST_AT:
                            post(s - 1)
                        if t == PRE_AT:
                            pre(jnp.minimum(s + 1, NSEG - 1), nxt)
                    if name == "qk" and 0 <= t - LAGS[0] < H:
                        st_qk(t - LAGS[0])
                    if name == "sm" and 0 <= t - LAGS[1] < H:
                        st_sm(t - LAGS[1])
                    if name == "pv" and 0 <= t - LAGS[2] < H:
                        st_pv(t - LAGS[2])
                    if name == "wo":
                        for g in WO_AT.get(t, []):
                            st_wo(g)
            y = ys[0]
            act_v[pl.ds(pl.multiple_of(nxt * LR, 8), M), :] = y[:M]
            y_v[...] = y[M:]

            @pl.when((s % OB == 0) & (s > 0))
            def _():
                cp_out(pl.multiple_of((s - OB) * SEG, OB * SEG), OB * SEG).start()

            return carry

        r_v[...] = jnp.zeros_like(r_v)
        y_v[...] = jnp.zeros_like(y_v)
        act_v[:M, :] = mem0_ref[...].astype(F32)
        pre(0, 0)
        jax.lax.fori_loop(0, NSEG, step, 0)
        post(NSEG - 1)
        cp_out((NSEG - OB) * SEG, OB * SEG).start()

        sb, cb, gb = mods(3), mods(4), mods(5)
        tok = lane * SEG + jax.lax.broadcasted_iota(jnp.int32, (SEG, 128), 0)
        rv = jnp.where(lane < NSEG, r_v[...], -jnp.inf)
        m0 = jnp.max(rv)
        i0 = jnp.min(jnp.where(rv == m0, tok, S - 1))
        rv1 = jnp.where(tok == i0, -jnp.inf, rv)
        m1 = jnp.max(rv1)
        i1 = jnp.min(jnp.where(rv1 == m1, tok, S - 1))
        row8 = jax.lax.broadcasted_iota(jnp.int32, (8, D), 0)
        xa = act_v[pl.ds(XO + SEG + i0, 1), :]
        xb = act_v[pl.ds(XO + SEG + i1, 1), :]
        x1s = jnp.where(row8 == 0, xa, jnp.where(row8 == 1, xb, 0.0))
        h2s = _rnd(_ln(x1s) * (1.0 + cb) + sb)
        cp_wg.wait()
        cp_wu.wait()
        cp_wd.wait()
        g = _dot(h2s, _w(wg_v[...]))
        u = _dot(h2s, _w(wu_v[...]))
        y = _dot(g * jax.nn.sigmoid(g) * u, _w(wd_v[...]))
        rsel = jnp.where(row8 == 0, m0, m1)
        y = y * jax.nn.sigmoid(rsel)
        fix = x1s + gb * (h2s + y)
        row16 = jax.lax.broadcasted_iota(jnp.int32, (16, D), 0)
        for n, idx in enumerate((i0, i1)):
            g0 = pl.multiple_of((idx // 16) * 16, 16)
            blk = out_v[pl.ds(g0 + SEG, 16), :].astype(F32)
            blk = jnp.where(row16 == idx - g0, fix[n:n + 1], blk)
            out_v[pl.ds(g0 + SEG, 16), :] = blk.astype(BF16)
        cp_out(0, S).wait()
        g0 = pl.multiple_of((i0 // 16) * 16, 16)
        g1 = pl.multiple_of((i1 // 16) * 16, 16)
        cp_out(g0, 16).start()

        @pl.when(g0 != g1)
        def _():
            cp_out(g1, 16).start()

        cp_out(g0, 16).wait()

        @pl.when(g0 != g1)
        def _():
            cp_out(g1, 16).wait()

    any_spec = pl.BlockSpec(memory_space=pl.ANY)
    vmem_spec = pl.BlockSpec(memory_space=pltpu.VMEM)
    out = pl.pallas_call(
        kernel,
        out_shape=jax.ShapeDtypeStruct((B * S, D), A_x.dtype),
        in_specs=[any_spec, vmem_spec, any_spec, any_spec, any_spec, any_spec, vmem_spec, vmem_spec,
                  any_spec, any_spec, any_spec, any_spec],
        out_specs=any_spec,
        scratch_shapes=[
            pltpu.VMEM((S, D), BF16),
            pltpu.VMEM((HP + 1, 3, 2, D // 2, E), U32),
            pltpu.VMEM((HE // 2, D), U32),
            pltpu.VMEM((D // 2, 6 * D), U32),
            pltpu.VMEM((D // 2, F), U32),
            pltpu.VMEM((D // 2, F), U32),
            pltpu.VMEM((F // 2, D), U32),
            pltpu.VMEM((RING, 3 * HE), F32),
            pltpu.VMEM((PRE, D), BF16),
            pltpu.VMEM((XO + S + SEG, D), F32),
            pltpu.VMEM((S + SEG, D), BF16),
            pltpu.VMEM((SEG, D), F32),
            pltpu.VMEM((8, 6 * D), F32),
            pltpu.VMEM((SEG, 128), F32),
            pltpu.SemaphoreType.DMA((9,)),
            pltpu.SemaphoreType.DMA((HP,)),
        ],
        compiler_params=pltpu.CompilerParams(vmem_limit_bytes=120 * 1024 * 1024, flags=FLAGS),
    )(
        A_x.reshape(B * S, D), A_mem0.reshape(B * M, D),
        A_Wq.reshape(D // 2, 2, H, E), A_Wk.reshape(D // 2, 2, H, E), A_Wv.reshape(D // 2, 2, H, E),
        A_Wo.reshape(HE, D), B_w_r, c, w_mod, B_w_gate, B_w_up, B_w_down,
    )
    return out.reshape(B, S, D)
```

```python
import functools

import jax
import jax.numpy as jnp
import jax.experimental.pallas as pl
import jax.experimental.pallas.tpu as pltpu

F32 = jnp.float32
BF16 = jnp.bfloat16
U32 = jnp.uint32

_NN = (((1,), (0,)), ((), ()))
_NT = (((1,), (1,)), ((), ()))


def _dot(a, b, dims=_NN):
    return jax.lax.dot_general(a, b, dims, preferred_element_type=F32)


def _w(v):
    return pltpu.bitcast(v, BF16)


def _rnd(v):
    return v.astype(BF16).astype(F32)


def _ln(v):
    m = jnp.mean(v, axis=-1, keepdims=True)
    d = v - m
    var = jnp.mean(d * d, axis=-1, keepdims=True)
    return d * jax.lax.rsqrt(var + 1e-05)


@functools.partial(jax.jit, static_argnames=("A_seg_len",))
def pallas_adaLN_cond__memory_aug_recurrent_mem_tr__moe_arch_mod__prompt_kernel(
    A_x: jax.Array,
    A_mem0: jax.Array,
    A_Wq: jax.Array,
    A_Wk: jax.Array,
    A_Wv: jax.Array,
    A_Wo: jax.Array,
    A_seg_len: jax.Array,
    B_x: jax.Array,
    B_w_r: jax.Array,
    B_w_gate: jax.Array,
    B_w_up: jax.Array,
    B_w_down: jax.Array,
    c: jax.Array,
    w_mod: jax.Array,
):
    B, S, D = A_x.shape
    _, H, E = A_Wq.shape
    M = A_mem0.shape[1]
    F = B_w_gate.shape[1]
    SEG = min(int(A_seg_len), S)
    NSEG = S // SEG
    L = M + SEG
    HE = H * E
    HP = H // 2
    scale = float(E) ** -0.5
    TPS = 24
    PRE = S - TPS * NSEG
    RING = 576
    SHIFT = RING - PRE
    LR = M + TPS
    XO = 2 * LR
    LAGS = (1, 2, 4)
    POST_AT = 1
    PRE_AT = 3
    WO_AT = {27: [(0, 8)], 31: [(8, 16)], 34: [(16, 24)], 35: [(24, 32)]}
    FLAGS = {'XLA_TPU_EVENLY_DISTRIBUTE_CRITICAL_NODES': True}
    PCH = 128
    OB = 8

    def kernel(x_hbm, mem0_ref, wq_hbm, wk_hbm, wv_hbm, wo_hbm, wr_ref, c_ref, wmod_hbm,
               wg_hbm, wu_hbm, wd_hbm, out_hbm,
               x_v, wqkv, wo_v, wmod_v, wg_v, wu_v, wd_v, ring, hpre, act_v, out_v, y_v, mod_v, r_v,
               sems, wsem):
        wmod32 = wmod_hbm.bitcast(U32)
        cp_mod1 = pltpu.make_async_copy(wmod32.at[:, pl.ds(0, 2 * D)], wmod_v.at[:, pl.ds(0, 2 * D)], sems.at[0])
        cp_mod2 = pltpu.make_async_copy(wmod32.at[:, pl.ds(2 * D, 4 * D)], wmod_v.at[:, pl.ds(2 * D, 4 * D)], sems.at[7])
        cp_x1 = pltpu.make_async_copy(x_hbm.at[pl.ds(0, PRE), :], x_v.at[pl.ds(0, PRE), :], sems.at[1])
        cp_x2 = pltpu.make_async_copy(x_hbm.at[pl.ds(PRE, S - PRE), :], x_v.at[pl.ds(PRE, S - PRE), :], sems.at[8])
        cp_wo = pltpu.make_async_copy(wo_hbm.bitcast(U32), wo_v, sems.at[2])
        cp_wg = pltpu.make_async_copy(wg_hbm.bitcast(U32), wg_v, sems.at[3])
        cp_wu = pltpu.make_async_copy(wu_hbm.bitcast(U32), wu_v, sems.at[4])
        cp_wd = pltpu.make_async_copy(wd_hbm.bitcast(U32), wd_v, sems.at[5])

        def cp_out(r0, n):
            return pltpu.make_async_copy(out_v.at[pl.ds(SEG + r0, n), :], out_hbm.at[pl.ds(r0, n), :], sems.at[6])

        srcs = tuple(w.bitcast(U32) for w in (wq_hbm, wk_hbm, wv_hbm))

        def wcps(hp):
            return [pltpu.make_async_copy(srcs[wi].at[:, p, hp, :], wqkv.at[hp, wi, p], wsem.at[hp])
                    for wi in range(3) for p in range(2)]

        def repack(hp):
            for wi in range(3):
                a = wqkv[hp, wi, 0]
                b = wqkv[hp, wi, 1]
                wqkv[hp, wi, 0] = (a & jnp.uint32(0xFFFF)) | (b << 16)
                wqkv[hp, wi, 1] = (a >> 16) | (b & jnp.uint32(0xFFFF0000))

        def whead(hp, hb):
            return _w(jnp.concatenate([wqkv[hp, wi, hb] for wi in range(3)], axis=1))

        cp_mod1.start()
        cp_x1.start()
        wqkv[HP] = jnp.zeros(wqkv.shape[1:], U32)

        def mods(i, n):
            return jnp.concatenate([mod_v[:, i * D:(i + 1) * D]] * (n // 8), axis=0)

        cs = c_ref[...].astype(F32)
        cs = jnp.broadcast_to(_rnd(cs * jax.nn.sigmoid(cs)), (8, D))
        cp_mod1.wait()
        for cp in wcps(0):
            cp.start()
        cp_x1.wait()
        mod_v[:, :2 * D] = _dot(cs, _w(wmod_v[:, :2 * D]))
        for cp in wcps(1):
            cp.start()

        def ada1(rows):
            n = rows.shape[0]
            return _ln(rows.astype(F32)) * (1.0 + mods(1, n)) + mods(0, n)

        def pre_ln(i, carry):
            r0 = pl.multiple_of(i * 64, 64)
            hpre[pl.ds(r0, 64), :] = ada1(x_v[pl.ds(r0, 64), :]).astype(BF16)
            return carry

        jax.lax.fori_loop(0, PRE // 64, pre_ln, 0)

        for cp in wcps(0):
            cp.wait()
        repack(0)

        def pre_proj(hp, carry):
            @pl.when(2 * hp + 2 < HP)
            def _():
                for cp in wcps(2 * hp + 2) + wcps(2 * hp + 3):
                    cp.start()

            for at, cps in ((HP // 2 + 2, (cp_wo, cp_x2, cp_mod2)),):
                @pl.when(hp == at)
                def _():
                    for cp in cps:
                        cp.start()

            @pl.when(hp + 1 < HP)
            def _():
                for cp in wcps(hp + 1):
                    cp.wait()

            repack(hp + 1)
            for hb in range(2):
                col = pl.multiple_of((2 * hp + hb) * 3 * E, 3 * E)
                for rc in range(PRE // PCH):
                    ring[pl.ds(SHIFT + rc * PCH, PCH), pl.ds(col, 3 * E)] = _dot(hpre[rc * PCH:(rc + 1) * PCH, :], whead(hp, hb))
            return carry

        jax.lax.fori_loop(0, HP, pre_proj, 0)

        cp_wg.start()
        cp_wu.start()
        cp_wd.start()
        cp_mod2.wait()
        mod_v[:, 2 * D:6 * D] = _dot(cs, _w(wmod_v[:, 2 * D:]))
        cp_wo.wait()
        cp_x2.wait()

        row = jax.lax.broadcasted_iota(jnp.int32, (L, L), 0)
        col = jax.lax.broadcasted_iota(jnp.int32, (L, L), 1)
        mask = (row < M) | (row >= col)
        lane = jax.lax.broadcasted_iota(jnp.int32, (SEG, 128), 1)

        def pre(s, slot):
            r0 = pl.multiple_of(PRE + s * TPS, 8)
            act_v[pl.ds(pl.multiple_of(slot * LR + M, 8), TPS), :] = ada1(x_v[pl.ds(r0, TPS), :])

        def post(s):
            rx = pl.multiple_of(jnp.maximum(s, 0) * SEG, SEG)
            r0 = pl.multiple_of((s + 1) * SEG, SEG)
            xs = x_v[pl.ds(rx, SEG), :].astype(F32)
            cb1 = 1.0 + mods(4, SEG)
            x1 = xs + mods(2, SEG) * y_v[...]
            h2 = _ln(x1) * cb1 + mods(3, SEG)
            wr = mods(6, SEG)
            r = _rnd(jnp.sum(h2 * wr, axis=-1, keepdims=True))
            r_v[...] = jnp.where(lane == s, r, r_v[...])
            act_v[pl.ds(XO + r0, SEG), :] = x1
            out_v[pl.ds(r0, SEG), :] = (x1 + mods(5, SEG) * h2).astype(BF16)

        def step(s, carry):
            cur = pl.multiple_of((s % 2) * LR, 8)
            nxt = 1 - s % 2
            wrow = pl.multiple_of((s * TPS) % RING, 8)
            rrow = pl.multiple_of((s * SEG + SHIFT) % RING, 8)
            qkv, sc, p, o = {}, {}, {}, {}
            lhs = act_v[pl.ds(cur, LR), :].astype(BF16)
            ys = [None]

            def st_qkv(t):
                cols = pl.ds(t * 3 * E, 3 * E)
                res = _dot(lhs, whead(t // 2, t % 2))
                ring[pl.ds(wrow, TPS), cols] = res[M:]
                qkv[t] = jnp.concatenate([res[:M], ring[pl.ds(rrow, SEG), cols]], axis=0)

            def st_qk(hh):
                sc[hh] = _dot(qkv[hh][:, :E], qkv[hh][:, E:2 * E], _NT)

            def st_sm(hh):
                z = jnp.where(mask, sc[hh] * scale, -1000000000.0)
                e = jnp.exp(z - jnp.max(z, axis=-1, keepdims=True))
                p[hh] = e / jnp.sum(e, axis=-1, keepdims=True)

            def st_pv(hh):
                o[hh] = _dot(p[hh], qkv[hh][:, 2 * E:])

            def st_wo(g):
                og = jnp.concatenate([o[i] for i in range(g[0], g[1])], axis=1)
                yg = _dot(og, _w(wo_v[g[0] * E // 2:g[1] * E // 2, :]))
                ys[0] = yg if ys[0] is None else ys[0] + yg

            for t in range(H + LAGS[2]):
                if t < H:
                    st_qkv(t)
                if t == POST_AT:
                    post(s - 1)
                if t == PRE_AT:
                    pre(jnp.minimum(s + 1, NSEG - 1), nxt)
                for lag, stage in zip(LAGS, (st_qk, st_sm, st_pv)):
                    if 0 <= t - lag < H:
                        stage(t - lag)
                for g in WO_AT.get(t, []):
                    st_wo(g)
            y = ys[0]
            act_v[pl.ds(pl.multiple_of(nxt * LR, 8), M), :] = y[:M]
            y_v[...] = y[M:]

            @pl.when((s % OB == 0) & (s > 0))
            def _():
                cp_out(pl.multiple_of((s - OB) * SEG, OB * SEG), OB * SEG).start()

            return carry

        r_v[...] = jnp.zeros_like(r_v)
        mod_v[:, 6 * D:] = jnp.broadcast_to(wr_ref[...].astype(F32).reshape(1, D), (8, D))
        y_v[...] = jnp.zeros_like(y_v)
        act_v[:M, :] = mem0_ref[...].astype(F32)
        pre(0, 0)
        jax.lax.fori_loop(0, NSEG, step, 0)
        post(NSEG - 1)
        cp_out((NSEG - OB) * SEG, OB * SEG).start()

        sb, cb, gb = mods(3, 8), mods(4, 8), mods(5, 8)
        tok = lane * SEG + jax.lax.broadcasted_iota(jnp.int32, (SEG, 128), 0)
        rv = jnp.where(lane < NSEG, r_v[...], -jnp.inf)
        m0 = jnp.max(rv)
        i0 = jnp.min(jnp.where(rv == m0, tok, S - 1))
        rv1 = jnp.where(tok == i0, -jnp.inf, rv)
        m1 = jnp.max(rv1)
        i1 = jnp.min(jnp.where(rv1 == m1, tok, S - 1))
        row8 = jax.lax.broadcasted_iota(jnp.int32, (8, D), 0)
        xa = act_v[pl.ds(XO + SEG + i0, 1), :]
        xb = act_v[pl.ds(XO + SEG + i1, 1), :]
        x1s = jnp.where(row8 == 0, xa, jnp.where(row8 == 1, xb, 0.0))
        h2s = _ln(x1s) * (1.0 + cb) + sb
        cp_wg.wait()
        cp_wu.wait()
        cp_wd.wait()
        g = _dot(h2s, _w(wg_v[...]))
        u = _dot(h2s, _w(wu_v[...]))
        y = _dot(g * jax.nn.sigmoid(g) * u, _w(wd_v[...]))
        rsel = jnp.where(row8 == 0, m0, m1)
        y = y * jax.nn.sigmoid(rsel)
        fix = x1s + gb * (h2s + y)
        cp_out(0, S).wait()
        row16 = jax.lax.broadcasted_iota(jnp.int32, (16, D), 0)
        for n, idx in enumerate((i0, i1)):
            g0 = pl.multiple_of((idx // 16) * 16, 16)
            blk = out_v[pl.ds(g0 + SEG, 16), :].astype(F32)
            blk = jnp.where(row16 == idx - g0, fix[n:n + 1], blk)
            out_v[pl.ds(g0 + SEG, 16), :] = blk.astype(BF16)
        g0 = pl.multiple_of((i0 // 16) * 16, 16)
        g1 = pl.multiple_of((i1 // 16) * 16, 16)
        cp_out(g0, 16).start()

        @pl.when(g0 != g1)
        def _():
            cp_out(g1, 16).start()

        cp_out(g0, 16).wait()

        @pl.when(g0 != g1)
        def _():
            cp_out(g1, 16).wait()

    any_spec = pl.BlockSpec(memory_space=pl.ANY)
    vmem_spec = pl.BlockSpec(memory_space=pltpu.VMEM)
    out = pl.pallas_call(
        kernel,
        out_shape=jax.ShapeDtypeStruct((B * S, D), A_x.dtype),
        in_specs=[any_spec, vmem_spec, any_spec, any_spec, any_spec, any_spec, vmem_spec, vmem_spec,
                  any_spec, any_spec, any_spec, any_spec],
        out_specs=any_spec,
        scratch_shapes=[
            pltpu.VMEM((S, D), BF16),
            pltpu.VMEM((HP + 1, 3, 2, D // 2, E), U32),
            pltpu.VMEM((HE // 2, D), U32),
            pltpu.VMEM((D // 2, 6 * D), U32),
            pltpu.VMEM((D // 2, F), U32),
            pltpu.VMEM((D // 2, F), U32),
            pltpu.VMEM((F // 2, D), U32),
            pltpu.VMEM((RING, 3 * HE), F32),
            pltpu.VMEM((PRE, D), BF16),
            pltpu.VMEM((XO + S + SEG, D), F32),
            pltpu.VMEM((S + SEG, D), BF16),
            pltpu.VMEM((SEG, D), F32),
            pltpu.VMEM((8, 7 * D), F32),
            pltpu.VMEM((SEG, 128), F32),
            pltpu.SemaphoreType.DMA((9,)),
            pltpu.SemaphoreType.DMA((HP,)),
        ],
        compiler_params=pltpu.CompilerParams(vmem_limit_bytes=120 * 1024 * 1024, flags=FLAGS),
    )(
        A_x.reshape(B * S, D), A_mem0.reshape(B * M, D),
        A_Wq.reshape(D // 2, 2, H, E), A_Wk.reshape(D // 2, 2, H, E), A_Wv.reshape(D // 2, 2, H, E),
        A_Wo.reshape(HE, D), B_w_r, c, w_mod, B_w_gate, B_w_up, B_w_down,
    )
    return out.reshape(B, S, D)
```
